```python
import os as _os
_os.environ.setdefault('JAX_PLATFORMS', 'cpu')
import jax
import jax.numpy as jnp

def _softmax(x, axis=-1):
    return jax.nn.softmax(x, axis=axis)

def _gelu(x):
    return jax.nn.gelu(x, approximate=True)

def _silu(x):
    return jax.nn.silu(x)

def _sigmoid(x):
    return jax.nn.sigmoid(x)

def _layernorm(x, axis=-1, eps=1e-05):
    m = jnp.mean(x, axis=axis, keepdims=True)
    v = jnp.var(x, axis=axis, keepdims=True)
    return (x - m) / jnp.sqrt(v + eps)

def _scatter_add(tgt, idx, src, axis=0):
    return tgt.at[idx].add(src)

def _segment_sum(src, seg, n):
    return jax.ops.segment_sum(src, seg, n)

class _Rng:

    def __init__(self, key):
        self._k = key

    def _next(self):
        self._k, sub = jax.random.split(self._k)
        return sub

    def normal(self, shape):
        return jax.random.normal(self._next(), shape, dtype=jnp.bfloat16)

    def randint(self, lo, hi, shape):
        return jax.random.randint(self._next(), shape, lo, hi, dtype=jnp.int32)

    def uniform(self, shape, lo=0.0, hi=1.0):
        return jax.random.uniform(self._next(), shape, jnp.bfloat16, lo, hi)

    def permutation(self, n):
        return jax.random.permutation(self._next(), n)
kernel_name = 'interleave_layers__memory_aug_recurrent_mem_tr__mixer_token_mlp__prompt'

def setup_inputs():
    _rng = _Rng(jax.random.key(int.from_bytes(__import__("os").urandom(4), "little")))
    _w = lambda a: (lambda t: t.astype(jnp.bfloat16) if jnp.issubdtype(t.dtype, jnp.floating) else t)(jnp.asarray(a))

    def _A_setup():
        B, S, Dm = (1, 2048, 640)
        H, Dh = (32, 128)
        M, seg = (8, 32)
        seg = min(seg, S)
        S = S // seg * seg
        return {'x': _w((lambda *s: _rng.normal(s) * 0.05)(B, S, Dm)), 'mem0': _w((lambda *s: _rng.normal(s) * 0.2)(B, M, Dm)), 'Wq': _w((lambda *s: _rng.normal(s) * 0.8)(Dm, H, Dh) * Dm ** (-0.5)), 'Wk': _w((lambda *s: _rng.normal(s) * 0.8)(Dm, H, Dh) * Dm ** (-0.5)), 'Wv': _w((lambda *s: _rng.normal(s) * 0.2)(Dm, H, Dh) * Dm ** (-0.5)), 'Wo': _w((lambda *s: _rng.normal(s) * 0.2)(H, Dh, Dm) * (H * Dh) ** (-0.5)), 'seg_len': seg}
    _A_in = _A_setup()

    def _B_setup():
        B, S, D, F = (1, 2048, 640, 1728)
        return {'x': _w((lambda *s: _rng.normal(s) * 0.05)(B, S, D)), 'w1': _w((lambda *s: _rng.normal(s) * 0.2)(S, F) * S ** (-0.5)), 'b1': _w((lambda *s: _rng.normal(s) * 0.2)(F) * 0.02), 'w2': _w((lambda *s: _rng.normal(s) * 0.2)(F, S) * F ** (-0.5)), 'b2': _w((lambda *s: _rng.normal(s) * 0.2)(S) * 0.02)}
    _B_in = _B_setup()
    return {'A_x': _A_in['x'], 'A_mem0': _A_in['mem0'], 'A_Wq': _A_in['Wq'], 'A_Wk': _A_in['Wk'], 'A_Wv': _A_in['Wv'], 'A_Wo': _A_in['Wo'], 'A_seg_len': _A_in['seg_len'], 'B_x': _B_in['x'], 'B_w1': _B_in['w1'], 'B_b1': _B_in['b1'], 'B_w2': _B_in['w2'], 'B_b2': _B_in['b2']}

def reference(A_x, A_mem0, A_Wq, A_Wk, A_Wv, A_Wo, A_seg_len, B_x, B_w1, B_b1, B_w2, B_b2):

    def _A_ref(x, mem0, Wq, Wk, Wv, Wo, seg_len):
        B, S, Dm = x.shape
        H, Dh = (Wq.shape[1], Wq.shape[2])
        M = mem0.shape[1]
        scale = Dh ** (-0.5)
        n_seg = S // seg_len
        L = M + seg_len
        idx = jnp.arange(L)
        mask = (idx[:, None] < M) | (idx[:, None] >= idx[None, :])
        mem = mem0
        outs = []
        for s in range(n_seg):
            xs = x[:, s * seg_len:(s + 1) * seg_len, :].copy()
            h = jnp.concatenate([mem, xs], axis=1)
            q = jnp.einsum('btd,dhe->bhte', h, Wq)
            k = jnp.einsum('btd,dhe->bhte', h, Wk)
            v = jnp.einsum('btd,dhe->bhte', h, Wv)
            scores = jnp.einsum('bhqe,bhke->bhqk', q, k) * scale
            scores = jnp.where(mask[None, None], scores, -1000000000.0)
            p = _softmax(scores, axis=-1)
            o = jnp.einsum('bhqk,bhke->bhqe', p, v)
            o = jnp.einsum('bhte,hed->btd', o, Wo)
            mem = o[:, :M, :].copy()
            outs.append(o[:, M:, :])
        return jnp.concatenate(outs, axis=1)

    def _B_ref(x, w1, b1, w2, b2):
        B, S, D = x.shape
        h = _layernorm(x, axis=-1)
        u = jnp.einsum('bsd,sf->bdf', h, w1) + b1
        u = _gelu(u)
        y = jnp.einsum('bdf,fs->bds', u, w2) + b2
        return (lambda x, *d: x.transpose(*d))(y, 0, 2, 1)
    x = A_x
    x = x + _A_ref(_layernorm(x, axis=-1), A_mem0, A_Wq, A_Wk, A_Wv, A_Wo, A_seg_len)
    x = x + _B_ref(_layernorm(x, axis=-1), B_w1, B_b1, B_w2, B_b2)
    x = x + _A_ref(_layernorm(x, axis=-1), A_mem0, A_Wq, A_Wk, A_Wv, A_Wo, A_seg_len)
    x = x + _B_ref(_layernorm(x, axis=-1), B_w1, B_b1, B_w2, B_b2)
    return x
```

```python
import functools

import jax
import jax.numpy as jnp
from jax import lax
import jax.experimental.pallas as pl
import jax.experimental.pallas.tpu as pltpu

F32, BF16, U32 = jnp.float32, jnp.bfloat16, jnp.uint32
NN = (((1,), (0,)), ((), ()))
NT = (((1,), (1,)), ((), ()))
EPS = 1e-5


def _ln(x):
    m = jnp.mean(x, axis=-1, keepdims=True)
    d = x - m
    v = jnp.mean(d * d, axis=-1, keepdims=True)
    return d * lax.rsqrt(v + EPS)


def _dot(a, b, dims=NN):
    return lax.dot_general(a, b, dims, preferred_element_type=F32)


def _kernel(x_hbm, mem0_ref, wq_hbm, wk_hbm, wv_hbm, wo_hbm, w1t_hbm, b1_ref, w2_hbm, b2_ref,
            out_hbm,
            xin, raw, wqkv, wo, w1t, w2, w2t, b1c, b2c, xres, hbuf, obuf, hb, gbuf, sems,
            *, S, DM, H, DH, M, SEG, F):
    L = M + SEG
    NSEG = S // SEG
    NJ = DM // 128
    scale = DH ** -0.5

    cx = pltpu.make_async_copy(x_hbm, xin, sems.at[0])
    cw = [pltpu.make_async_copy(w.bitcast(U32), raw.at[i], sems.at[1 + i]) for i, w in enumerate((wq_hbm, wk_hbm, wv_hbm))]
    wo_u32 = wo_hbm.bitcast(U32)
    co = [pltpu.make_async_copy(wo_u32.at[:, pl.ds(j * 128, 128)], wo.at[j], sems.at[4 + j]) for j in range(NJ)]
    c1 = pltpu.make_async_copy(w1t_hbm, w1t, sems.at[9])
    c2 = pltpu.make_async_copy(w2_hbm, w2, sems.at[10])
    for c in [cx] + cw + co + [c1, c2]:
        c.start()

    cx.wait()

    def init_x(i, _):
        r = pl.multiple_of(i * 128, 128)
        xres[pl.ds(r, 128), :] = xin[pl.ds(r, 128), :].astype(F32)
        return 0
    lax.fori_loop(0, S // 128, init_x, 0)

    HP = H // 2
    for i in range(3):
        cw[i].wait()
        src = raw.at[i]

        def repack(db, _, i=i, src=src):
            base = db * (16 * HP)
            ro = pl.multiple_of(db * 8, 8)
            for hp in range(HP):
                a = src[pl.ds(base + hp, 8, stride=2 * HP), :]
                b = src[pl.ds(base + HP + hp, 8, stride=2 * HP), :]
                wqkv[3 * (2 * hp) + i, pl.ds(ro, 8), :] = (a & 0xFFFF) | (b << 16)
                wqkv[3 * (2 * hp + 1) + i, pl.ds(ro, 8), :] = (a >> 16) | (b & jnp.uint32(0xFFFF0000))
            return 0
        lax.fori_loop(0, DM // 16, repack, 0)
    for c in co:
        c.wait()

    r_i = lax.broadcasted_iota(jnp.int32, (L, L), 0)
    c_i = lax.broadcasted_iota(jnp.int32, (L, L), 1)
    mask = (r_i < M) | (r_i >= c_i)
    LAG1, LAG2, OCH = 2, 5, 4

    def a_step(s, _):
        r0 = pl.multiple_of(s * SEG, SEG)
        rn = pl.multiple_of(jnp.minimum(s + 1, NSEG - 1) * SEG, SEG)
        rp = pl.multiple_of(jnp.maximum(s - 1, 0) * SEG, SEG)
        h_next = _ln(xres[pl.ds(rn, SEG), :]).astype(BF16).astype(F32)
        hb[pl.ds(rp, SEG), :] = _ln(_ln(xres[pl.ds(rp, SEG), :])).astype(BF16)
        qkv, ps = {}, {}

        def do_qkv(h):
            w = jnp.concatenate([pltpu.bitcast(wqkv[3 * h + j], BF16) for j in range(3)], axis=1)
            y = _dot(hbuf[...], w)
            qkv[h] = tuple(y[:, j * DH:(j + 1) * DH] for j in range(3))

        def do_s(h):
            q, k, v = qkv[h]
            sc = _dot(q, k.astype(BF16), NT)
            sc = jnp.where(mask, sc * scale, -1e9)
            e = jnp.exp(sc - jnp.max(sc, axis=-1, keepdims=True))
            ps[h] = (e, jnp.sum(e, axis=-1, keepdims=True), v.astype(BF16))

        def do_pv(h):
            e, l, v = ps[h]
            obuf[:, h * DH:(h + 1) * DH] = _dot(e, v) / l

        acc = []

        def do_o(h0):
            w = jnp.concatenate(
                [pltpu.bitcast(wo[j, h0 * DH // 2:(h0 + OCH) * DH // 2, :], BF16) for j in range(NJ)], axis=1)
            y = _dot(obuf[:, h0 * DH:(h0 + OCH) * DH], w)
            acc[:] = [y + acc[0]] if acc else [y]

        och = list(range(0, H, OCH))
        for g in range(H + LAG2):
            if g < H:
                do_qkv(g)
            elif och:
                do_o(och.pop(0))
            if 0 <= g - LAG1 < H:
                do_s(g - LAG1)
            if 0 <= g - LAG2 < H:
                do_pv(g - LAG2)
        for h0 in och:
            do_o(h0)
        y = acc[0]
        hbuf[0:M, :] = y[0:M]
        hbuf[M:L, :] = h_next
        xres[pl.ds(r0, SEG), :] += y[M:L]
        return 0

    FC, SC = 288, 256

    def layer(it, _):
        hbuf[0:M, :] = mem0_ref[...].astype(F32)
        hbuf[M:L, :] = _ln(xres[0:SEG, :]).astype(BF16).astype(F32)
        lax.fori_loop(0, NSEG, a_step, 0)
        hb[S - SEG:S, :] = _ln(_ln(xres[S - SEG:S, :])).astype(BF16)

        @pl.when(it == 0)
        def _():
            c1.wait()
            c2.wait()
            b1c[...] = jnp.broadcast_to(b1_ref[...].astype(F32), (128, F)).T
            b2c[...] = jnp.broadcast_to(b2_ref[...].astype(F32), (128, S)).T

            def tr(i, _):
                c = pl.multiple_of(i * 128, 128)
                w2t[pl.ds(c, 128), :] = w2[:, pl.ds(c, 128)].T
                return 0
            lax.fori_loop(0, S // 128, tr, 0)

        def b_up(i, _):
            r = pl.multiple_of(i * FC, 16)
            u = _dot(w1t[pl.ds(r, FC), :], hb[...])
            u = u + jnp.tile(b1c[pl.ds(r, FC), :], (1, NJ))
            gbuf[pl.ds(r, FC), :] = jax.nn.gelu(u, approximate=True).astype(BF16)
            return 0
        lax.fori_loop(0, F // FC, b_up, 0)

        def b_down(i, _):
            r = pl.multiple_of(i * SC, SC)
            y = _dot(w2t[pl.ds(r, SC), :], gbuf[...])
            xres[pl.ds(r, SC), :] += y + jnp.tile(b2c[pl.ds(r, SC), :], (1, NJ))
            return 0
        lax.fori_loop(0, S // SC, b_down, 0)
        return 0

    lax.fori_loop(0, 2, layer, 0)

    def fin(i, _):
        r = pl.multiple_of(i * 128, 128)
        xin[pl.ds(r, 128), :] = xres[pl.ds(r, 128), :].astype(BF16)
        return 0
    lax.fori_loop(0, S // 128, fin, 0)
    cout = pltpu.make_async_copy(xin, out_hbm, sems.at[0])
    cout.start()
    cout.wait()


@functools.partial(jax.jit, static_argnames=("A_seg_len",))
def pallas_interleave_layers__memory_aug_recurrent_mem_tr__mixer_token_mlp__prompt_kernel(
    A_x, A_mem0, A_Wq, A_Wk, A_Wv, A_Wo, A_seg_len, B_x, B_w1, B_b1, B_w2, B_b2,
):
    del B_x
    B, S, DM = A_x.shape
    H, DH = A_Wq.shape[1:]
    M = A_mem0.shape[1]
    F = B_w1.shape[1]
    SEG = int(A_seg_len)
    L = M + SEG
    assert B == 1
    hbm = pl.BlockSpec(memory_space=pl.ANY)
    vmem = pl.BlockSpec(memory_space=pltpu.VMEM)
    out = pl.pallas_call(
        functools.partial(_kernel, S=S, DM=DM, H=H, DH=DH, M=M, SEG=SEG, F=F),
        out_shape=jax.ShapeDtypeStruct((S, DM), A_x.dtype),
        in_specs=[hbm, vmem, hbm, hbm, hbm, hbm, hbm, vmem, hbm, vmem],
        out_specs=hbm,
        scratch_shapes=[
            pltpu.VMEM((S, DM), BF16),
            pltpu.VMEM((3, DM * H // 2, DH), U32),
            pltpu.VMEM((3 * H, DM // 2, DH), U32),
            pltpu.VMEM((DM // 128, H * DH // 2, 128), U32),
            pltpu.VMEM((F, S), BF16),
            pltpu.VMEM((F, S), BF16),
            pltpu.VMEM((S, F), BF16),
            pltpu.VMEM((F, 128), F32),
            pltpu.VMEM((S, 128), F32),
            pltpu.VMEM((S, DM), F32),
            pltpu.VMEM((L, DM), F32),
            pltpu.VMEM((L, H * DH), F32),
            pltpu.VMEM((S, DM), BF16),
            pltpu.VMEM((F, DM), BF16),
            pltpu.SemaphoreType.DMA((11,)),
        ],
        compiler_params=pltpu.CompilerParams(vmem_limit_bytes=120 * 2**20),
        name="rmt_mixer",
    )(
        A_x.reshape(S, DM), A_mem0.reshape(M, DM),
        A_Wq.reshape(DM * H, DH), A_Wk.reshape(DM * H, DH), A_Wv.reshape(DM * H, DH),
        A_Wo.reshape(H * DH, DM), B_w1.T, B_b1.reshape(1, F), B_w2, B_b2.reshape(1, S),
    )
    return out.reshape(B, S, DM)
```

```python
import functools

import jax
import jax.numpy as jnp
from jax import lax
import jax.experimental.pallas as pl
import jax.experimental.pallas.tpu as pltpu

F32, BF16, U32 = jnp.float32, jnp.bfloat16, jnp.uint32
NN = (((1,), (0,)), ((), ()))
NT = (((1,), (1,)), ((), ()))
EPS = 1e-5

LAM = (0.0, -0.5, 0.5, 1.5, -1.5)
MLAM = (-1.375, -0.3125, 0.3125, 1.375)
NB, MB = len(LAM), len(MLAM)
PAIRS = tuple((k, l) for k in range(NB) for l in range(k + 1, NB))
ORDER = tuple(p for k in range(NB) for p in [q[::d] for q in PAIRS if q[0] == k for d in (1, -1)] + [(k, k)])
FEEDS = PAIRS + tuple((l,) for l in range(NB))
NLONG = len(FEEDS)
BUNDLE = 4
HEAD = 3
LATE = 6
STORES = (0, 10, 13, 14, 15, 16)

BUNDLE_SCHEDULE = dict(
    blocks="q0 k0 q1 k1 v0 q2 k2 v1 q3 k3 v2 o0 q4 k4 v3 o1 q5 k5 v4 v5 o2 o3 o4 o5",
    plain_pace=2, values_lag=12, rounds=(
        "lmmmmlmmmmlmmmmlmmmmlmmxmmmlmmmmxmlmmmmlmmmxmmammmxmammmxmxmammmxmmammmammmammmmlmmmmlmmmmlmmmmxmlmm"
        "mmammmammmmlmmmmlmmmmlmmmmlmmmmlmmmmlmmmmammmammmammmxmmammmammmammmmlmmmmammmammmmlmmmmlmmmlmmmmxl",
        "lmmmmlmmmmlmmmmlmmmmlmmxmmmlmmmmxmlmmmmlmmmxmmammmaxmmmmxmxmammmxmmammmammmammmammmmlmmmmlmmmmxmlmmm"
        "mlmmmmlmmmmlmmmmammmammmammmammmmlmmmmlmmmmlmmmmlmmmmammmammxmmammmmlmmmammmmammmmlmmmmlmmmmlmmmmx",
        "llmmmmlmmmmlmmmmlmmmmlmmxmmmlmmmmxmlmmmmlmmmxmmxmlmmmmammmammmxmxmxmammmmammmammmammmmlmmmmlmmmmxmam"
        "mmmammmlmmmmlmmmmlmmmmlmmmmlmmmmlmmmmlmmmmammmammmammmxmmammmammmammmmlmmmmammmammmmlmmmmlmmmmlmmmx",
        "llmmmmlmmmmlmmmmxmxmxmxmmammlmmmmlmmmmaxmmmmlmmmmammammmmlmmmmxmxmmmammxmammmmammmlmmmmlmmmmlmmmmlmm"
        "mmlmmmmlmmmmlmmmmammmammmammmammmmlmmmmlmmmmlmmmmlmmmmammmammmmlmmmmammmammmmlmmmmammmxmmlmmmmxmmm",
    ))
HEAD_SCHEDULE = dict(
    blocks="q0 k0 v0 q1 k1 v1 q2 k2 v2 q3 k3 v3 q4 k4 q5 k5 v4 v5",
    plain_pace=1, values_lag=8, rounds=(
        "xmxmxmxxmmxmxmmmmmmmmmmmmammmmmmmmmammmmmxmmammmmammmmmxmxmxmmammxmxmxmxmmmmammmamxmxmmxmxmmammmmmxx"
        "xmxmmammmxxmmxmxmmammmxxmmxmmmmmammmamxmmmxmxxmmxmmammmmmmammmaxxxaxxxxxxxxxx",
    ))


def _ln(x, axis=-1, twice=False):
    m = jnp.mean(x, axis=axis, keepdims=True)
    d = x - m
    v = jnp.mean(d * d, axis=axis, keepdims=True)
    r = lax.rsqrt(v + EPS)
    if twice:
        r = r * lax.rsqrt(v * r * r + EPS)
    return d * r


def _dot(a, b, dims=NN):
    return lax.dot_general(a, b, dims, preferred_element_type=F32)


def _pack(x):
    return pltpu.bitcast(x.astype(BF16), U32)


def _unpack(w):
    return pltpu.bitcast(w, BF16)


def _ev(t, l):
    g = t.shape[0] // 2
    return t[g:] + LAM[l] * t[:g] if LAM[l] else t[g:]


def _long_operand(t, j):
    if j >= len(PAIRS):
        x = t(j - len(PAIRS))
        return x[:x.shape[0] // 2]
    k, l = PAIRS[j]
    return _ev(t(l), l) - _ev(t(k), k)


def _add(d, key, v):
    d[key] = d[key] + v if key in d else v


def _mixer_lhs(t):
    g = t[0].shape[0] // 2
    ev = {(k, l): t[k][g:] + MLAM[l] * t[k][:g] for k in range(MB) for l in range(MB)}
    out = {}
    for l in range(MB):
        out["p", l, l] = t[l][:g]
        out["r", l, l] = ev[l, l]
        for k in range(MB):
            if k != l:
                out["r", k, l] = ev[k, l] - ev[l, l]
            if k < l:
                out["m", k, l] = ev[l, l] - ev[k, k]
    return {key: v.astype(BF16) for key, v in out.items()}


def _mixer_product(lhs, w, dims, keep, done, first=False):
    def prod(key, terms):
        acc = None
        for kt, a in enumerate(lhs):
            ws = [(c, x) for c, x in ((c, w(kt, k, l)) for c, k, l in terms) if x is not None]
            if not ws:
                continue
            c0, b = ws[0]
            if len(ws) > 1 or c0 != 1:
                b = b.astype(F32)
                for c, x in ws[1:]:
                    b = b + x.astype(F32) if c == c0 else b - x.astype(F32)
                b = (b if c0 == 1 else b * c0).astype(BF16)
            r = _dot(a[key], b, dims)
            acc = r if acc is None else acc + r
        return acc

    u, z = {}, {}
    p_prod = lambda k: prod(("p", k, k), [(1, k, k)] + [(-1, k, l) for l in range(MB) if l != k])
    z_prod = lambda k: prod(("r", k, k), [(1, l, k) for l in range(MB)])
    finish = lambda k, zk: done(k, jnp.concatenate([u[k](), zk - MLAM[k] * u[k]()], axis=0))

    def bump(acc, base, l, v):
        acc[l] = keep(base + l, acc[l]() + v if l in acc else v)

    def pair(k, l):
        c = 1.0 / (MLAM[l] - MLAM[k])
        r = prod(("r", l, k), [(1, l, k)])
        if r is None:
            return
        bump(z, MB, k, r)
        rest = keep(2 * MB, r)
        r = prod(("r", k, l), [(1, k, l)])
        bump(z, MB, l, r)
        rest = keep(2 * MB + 1, (r - rest()) * c)
        d = rest() + prod(("m", k, l), [(c, k, l), (c, l, k)])
        bump(u, 0, l, d)
        bump(u, 0, k, d)

    if first:
        for l in range(MB):
            bump(u, 0, l, p_prod(l))
            yield
            bump(z, MB, l, z_prod(l))
            yield
            for k in range(l):
                pair(k, l)
                if l == MB - 1:
                    finish(k, z[k]())
                yield
        finish(MB - 1, z[MB - 1]())
    else:
        for k in range(MB):
            for l in range(k + 1, MB):
                pair(k, l)
            bump(u, 0, k, p_prod(k))
            finish(k, z_prod(k) + z[k]())


def _queues(H, blocks, plain_pace, values_lag, rounds):
    NU = H // NB
    names = blocks.split()
    main = [("main", n[0], int(n[1:]), kl) for n in names for kl in ORDER]
    fast = lambda kind, h: "%s%d" % (kind, h // NB) in names
    heads = list(range(NU * NB, H)) + list(range(NU * NB))
    plain = [("plain", t, h, k) for h in heads for t in range(3) if not fast("qkv"[t], h) for k in range(NB)]
    plain += [("out", h, l) for h in heads if not fast("o", h) for l in range(NB)]
    source, when = {}, {}
    for ops, pace in ((main, 1), (plain, len(main) / len(plain) / plain_pace)):
        for n, op in enumerate(ops):
            if op[0] == "main" and op[1] != "o" and op[3][0] == op[3][1]:
                key = ("qkv".index(op[1]), op[2] * NB + op[3][0])
            elif op[0] == "plain":
                key = op[1:3]
            else:
                continue
            source[key], when[key] = op, n // 4 * pace
    att = [(max(when[0, h], when[1, h]), "scores", h) for h in range(H)]
    att += [(max(when[2, h], att[h][0] + values_lag), "values", h) for h in range(H)]
    pool, att = [a[1:] for a in sorted(att)], []
    while pool:
        att += [op for op in pool if op[0] == "scores" or ("scores", op[1]) in att][:4]
        pool = [op for op in pool if op not in att]

    def after(op):
        if op[0] == "scores":
            return [source[0, op[1]], source[1, op[1]]]
        if op[0] == "values":
            return [source[2, op[1]], ("scores", op[1])]
        if op[0] == "out":
            return [("values", op[1])]
        if op[:2] == ("main", "o"):
            return [("values", op[2] * NB + k) for k in range(NB)]
        return []

    longs = []
    if len(rounds) > 1:
        qkv = [n for n in names if n[0] != "o"]
        groups = [range(u, u + 2) for u in range(0, NU, 2)]
        longs = [("long_out", j, u, g) for g in groups[1:] for j in range(NLONG) for u in g]
        longs += [("long", "qkv".index(n[0]) * NU + int(n[1:]), j)
                  for t in range(BUNDLE - 1) for n in qkv[t::BUNDLE - 1] for j in range(NLONG)]
        longs += [("long_out", j, u, groups[0]) for j in range(NLONG) for u in groups[0]]
    return main, att, plain, longs, after


def _program(H, schedule):
    main, att, plain, longs, after = _queues(H, **schedule)
    longs, prog, phase = iter(longs), [], {}
    for i, seq in enumerate(schedule["rounds"]):
        src = {"m": iter(main), "a": iter(att), "x": iter(plain), "l": longs}
        ops = [op for op in (next(src[kind], None) for kind in seq for _ in range(4)) if op]
        assert all(next(src[kind], None) is None for kind in "max")
        seen, used = set(), set()
        for op in ops:
            assert all(dep in seen for dep in after(op))
            seen.add(op)
            if op[0] == "main" and op[1] != "o" and op[3][0] >= op[3][1]:
                used.add(("qkv".index(op[1]) * (H // NB) + op[2], FEEDS.index(tuple(sorted(set(op[3]))))))
            if op[0] == "long_out":
                assert all((("values", op[2] * NB + l) in seen) == (op[3][0] == 0) for l in range(NB))
                assert i == (BUNDLE - 1 if op[3][0] == 0 else 0)
            if op[0] == "long":
                phase[op[1:]] = i + (op[1:] in used)
        prog.append(ops)
    assert next(longs, None) is None
    return prog, phase


def _kernel(x_hbm, mem0_hbm, wq_hbm, wk_hbm, wv_hbm, wo_hbm, w1t_hbm, b1_hbm, w2_hbm, b2_hbm,
            out_hbm,
            xio, xres, xmid, hx, ml, wr, wo, wb, wd, wdo, ahead, part, opart, memb, xm, xt, qkv, eb, ob, spare,
            ymid, hb, macc, mem0_ref, b1_ref, b2_ref, sems):
    S, DM = xres.shape
    M = memb.shape[0]
    H, L, DH = qkv[0].shape
    F = w2_hbm.shape[0]
    SEG = L - M
    G = SEG // 2
    NSEG = S // SEG
    NBUN = NSEG // BUNDLE
    NU = H // NB
    NG = NU // 2
    NN2 = NB * NB
    scale = DH ** -0.5
    tile = lambda j: slice(j * 128, (j + 1) * 128)
    prog, phase = _program(H, BUNDLE_SCHEDULE)
    (head_prog,), _ = _program(H, HEAD_SCHEDULE)
    lane0 = jnp.minimum(pl.program_id(0), 0)

    def rows_at(r0, n):
        return pl.ds(r0 if isinstance(r0, int) else pl.multiple_of(r0, n), n)

    def park(ref, idx, val):
        pltpu.store(ref.at[idx], val, mask=lax.broadcasted_iota(jnp.int32, val.shape, 1) >= lane0)

    def hold(ref, n, val):
        idx = (n, slice(0, val.shape[0]))
        park(ref, idx, val)
        return lambda: ref[idx]

    def prep_tokens(s, x):
        h = _ln(x)
        hx[rows_at(s * SEG, SEG), :] = h
        for j in range(NLONG):
            ml[j, rows_at(s * (G // 2), G // 2), :] = _pack(_long_operand(lambda k: h[:, tile(k)], j))

    def prep_step(s, slot):
        rows = rows_at(jnp.minimum(s, NSEG - 1) * SEG, SEG)
        for l in range(NB):
            e = [_ev(hx[rows, tile(k)], l) for k in range(NB)]
            for k in range(NB):
                xt[slot * NN2 + k * NB + l] = e[k] - e[l] if k != l else e[l]

    def combine(get, put_long, put_diag):
        w = lambda k, l: _unpack(get(k, l)).astype(F32)
        csum = [w(l, l) for l in range(NB)]
        rdif = list(csum)
        for j, (k, l) in enumerate(PAIRS):
            wkl, wlk = w(k, l), w(l, k)
            put_long(j, _pack((wkl + wlk) * (1.0 / (LAM[l] - LAM[k]))))
            csum[l], csum[k] = csum[l] + wkl, csum[k] + wlk
            rdif[k], rdif[l] = rdif[k] - wkl, rdif[l] - wlk
        for l in range(NB):
            put_long(len(PAIRS) + l, _pack(rdif[l]))
            put_diag(l, _pack(csum[l]))

    def combine_out(r):
        u, rows = r // 8, rows_at(r % 8 * 8, 8)

        def put_long(j, v):
            wb[(3 * NU + u) * NLONG + j, rows, :] = v

        def put_diag(l, v):
            wdo[u * NB + l, rows, :] = v
        combine(lambda k, l: wo[l, rows_at((u * NB + k) * 64 + r % 8 * 8, 8), :], put_long, put_diag)

    def start_up(raw, acc, mlh, stage):
        T0 = HEAD + 1
        TC = pl.cdiv(NBUN - T0, 6)
        x_count = [max(min(TC, NBUN - T0 - c * TC), 0) for c in range(6)]

        def x_copy(lo, n, sem):
            rows = pl.ds(lo * 128, n * 128)
            return pltpu.make_async_copy(x_hbm.at[rows], xio.at[rows], sems.at[sem])
        x_copy(0, T0, 0).start()
        for c in range(6):
            if x_count[c]:
                x_copy(T0 + c * TC, x_count[c], 7 + c).start()
            w = (wq_hbm, wk_hbm, wv_hbm)[c // 2].bitcast(U32)
            pltpu.make_async_copy(w.at[:, pl.ds(c % 2 * 8, 8)], raw.at[pl.ds(c * DM, DM)], sems.at[1 + c]).start()
        wo_loads = [pltpu.make_async_copy(wo_hbm.bitcast(U32).at[r, tile(l)], wo.at[l, r], sems.at[13 + g * NB + l])
                    for g, r in enumerate((pl.ds(0, H * 32), pl.ds(H * 32, H * 32))) for l in range(NB)]
        wo_loads.append(pltpu.make_async_copy(mem0_hbm, mem0_ref, sems.at[13 + 2 * NB]))
        for c in wo_loads:
            c.start()
        for ref in (ob, opart, ymid, stage[-1]):
            ref[...] = jnp.zeros(ref.shape, ref.dtype)
        xmid[tile(0), :] = jnp.zeros((128, DM), F32)
        ml[:, S // 4:, :] = jnp.zeros((NLONG, BUNDLE * G // 2, 128), U32)

        def init_x(t, _):
            xs = xio[rows_at(t * 128, 128), :].astype(F32)
            xres[rows_at(t * 128, 128), :] = xs
            for i in range(BUNDLE):
                prep_tokens(t * BUNDLE + i, xs[i * SEG:(i + 1) * SEG])
            return 0
        x_copy(0, T0, 0).wait()
        lax.fori_loop(0, T0, init_x, 0)
        mlh[...] = ml[:, :mlh.shape[1], :]
        for ref in (xm, spare, macc, acc, *qkv, *stage[:-1]):
            ref[...] = jnp.zeros(ref.shape, ref.dtype)

        def long_ahead(b, slot):
            n = HEAD * BUNDLE * G
            long_w, sums_out = wb.at[pl.ds(b * NLONG, NLONG)], ahead.at[pl.ds(b * NB, NB)]
            parts = part.at[pl.ds(b * NLONG * BUNDLE, NLONG * BUNDLE)]
            seen = [0] * NB
            for js in ((0, 1, 2, 3), (4, 5, 6, 11), (7, 8, 12, 10), (9, 13, 14)):
                sums = {}
                for j in js:
                    w = stage[slot][j]
                    long_w[j] = w
                    y = _dot(_unpack(mlh[j]), _unpack(w))
                    for q in range(BUNDLE):
                        parts[j * BUNDLE + q] = y[n + q * G:n + (q + 1) * G]
                    for l in FEEDS[j]:
                        _add(sums, l, y[:n])
                for l, v in sums.items():
                    v = acc[l] + v if seen[l] else v
                    seen[l] += sum(l in FEEDS[j] for j in js)
                    if seen[l] == NB:
                        sums_out[l] = v
                    else:
                        park(acc, l, v)

        words = raw.reshape(raw.shape[0] * 8, DH)

        def half(c, _):
            for n in range(6):
                if x_count[n]:
                    pl.when(c == n)(x_copy(T0 + n * TC, x_count[n], 7 + n).wait)
            part_c = raw.at[pl.ds(c * DM, DM)]
            pltpu.make_async_copy(part_c, part_c, sems.at[1 + c]).wait()

            def repack(r, _):
                rows = rows_at(r % 8 * 8, 8)
                for hp in range(8):
                    at = (c * (DM // 16) + r) * 128 + hp
                    w = jnp.concatenate([words[pl.ds(at + p * 64, 8, stride=8), :] for p in range(2)], axis=0)
                    for h, v in ((2 * hp, w << 16), (2 * hp + 1, w & jnp.uint32(0xFFFF0000))):
                        wr[(c * 16 + h) * NB + r // 8, rows, :] = _pack(pltpu.bitcast(v, F32))
                return 0
            lax.fori_loop(0, DM // 16, repack, 0, unroll=2)

            plain = wr.at[pl.ds((c // 2 * H + c % 2 * NG * NB) * NB, NG * NN2)]
            diag_w = wd.at[pl.ds(c * NG * NB, NG * NB)]
            for b in range(NG):
                long_ahead(jnp.maximum(c * NG + b - 1, 0), b - 1)
                for r in (slice(r, r + 8) for r in range(0, 64, 8)):
                    def put_diag(l, v):
                        diag_w[b * NB + l, r, :] = v
                    combine(lambda k, l: plain[(b * NB + l) * NB + k, r, :],
                            lambda j, v: park(stage[b], (j, r), v), put_diag)
            for t in range(TC):
                init_x(jnp.minimum(T0 + c * TC + t, NBUN - 1), 0)
            return 0
        lax.fori_loop(0, 6, half, 0)

        for c in wo_loads[:NB]:
            c.wait()
        long_ahead(3 * NU - 1, NG - 1)
        for r in range(NG * 8):
            combine_out(r)
        for c in wo_loads[NB:]:
            c.wait()

    pl.run_scoped(
        start_up, pltpu.VMEM((6 * DM + 1, 8, DH), U32), pltpu.VMEM((NB, HEAD * BUNDLE * G, 128), F32),
        pltpu.VMEM((NLONG, (HEAD + 1) * BUNDLE * G // 2, 128), U32), [pltpu.VMEM((NLONG, 64, 128), U32)] * NG)

    r_i = lax.broadcasted_iota(jnp.int32, (L, L), 0)
    c_i = lax.broadcasted_iota(jnp.int32, (L, L), 1)
    mask = (r_i < M) | (r_i >= c_i)

    def long_qkv(seg0, ph, n, b, j):
        r0 = (seg0 + ph) * (G // 2)
        rows = pl.ds(r0 if isinstance(r0, int) else pl.multiple_of(r0, G // 2), n * G // 2)
        y = _dot(_unpack(ml[j, rows, :]), _unpack(wb[b * NLONG + j]))
        for s in range(ph, ph + n):
            idx = (b * NLONG + j) * BUNDLE + s % BUNDLE
            if s < BUNDLE and not isinstance(seg0, int):
                park(part, idx, y[(s - ph) * G:(s - ph + 1) * G])
            else:
                part[idx] = y[(s - ph) * G:(s - ph + 1) * G]

    def long_out(t, acc, j, u, group):
        lhs = [_long_operand(lambda k: ob[i * H + u * NB + k, M:, :], j) for i in range(BUNDLE)]
        _add(acc, j, _dot(jnp.concatenate(lhs, axis=0).astype(BF16), _unpack(wb[(3 * NU + u) * NLONG + j])))
        if u != group[-1]:
            return
        y = acc.pop(j)
        for l in FEEDS[j]:
            fresh = group[0] == 0 and j == min(n for n, f in enumerate(FEEDS) if l in f)
            opart[l] = y if fresh else opart[l] + y
        if u == NU - 1 and j == NLONG - 1:
            cols = []
            for l in range(NB):
                ys = [opart[l, i * G:(i + 1) * G, :] for i in range(BUNDLE)]
                cols.append(ymid[:, tile(l)] + jnp.concatenate([v for y in ys for v in (y, -LAM[l] * y)], axis=0))
            x = jnp.concatenate(cols, axis=1)
            xmid[rows_at(t * 128, 128), :] = x
            hb[t] = x.T

    def step(s, i, ops, extra):
        rows = rows_at(s * SEG, SEG)
        mem = [memb[:, tile(k)] for k in range(NB)]
        lhs_mem = {(k, l): hold(xm, k * NB + l, mem[k] - mem[l] if k != l else mem[l]) for k, l in ORDER}
        z, u1, tmp = {}, {}, {}
        fetch = lambda v: v() if callable(v) else v

        def main(kind, u, kl):
            k, l = kl
            if kind == "o":
                key, lhs, h = "o", tmp["o", u, k, l], u * NB + k
                w = wo[l, h * 64:(h + 1) * 64, :] if k != l else wdo[u * NB + l]
            else:
                t = "qkv".index(kind)
                key = b = t * NU + u
                lhs = jnp.concatenate([lhs_mem[kl](), xt[(i or 0) * NN2 + k * NB + l]], axis=0)
                w = wr[(t * H + u * NB + l) * NB + k] if k != l else wd[b * NB + l]
            r = _dot(lhs, _unpack(w))
            z[key, l] = fetch(z[key, l]) + r if (key, l) in z else r
            if k < l:
                tmp["r", key] = r
            elif k > l:
                d = tmp["r", key][M:] - r[M:]
                c = 1.0 / (LAM[k] - LAM[l])
                d = d * c if c != 1.0 else d
                if kind != "o" and i is not None:
                    d = d + part[(b * NLONG + PAIRS.index((l, k))) * BUNDLE + i]
                for n in (l, k):
                    u1[key, n] = fetch(u1[key, n]) + d if (key, n) in u1 else d
            elif kind == "o":
                if u < NU - 1:
                    z[key, l] = hold(spare, l, z[key, l])
                    u1[key, l] = hold(spare, NB + l, u1[key, l])
            else:
                if i is None:
                    y1 = u1[key, l] + ahead[b * NB + l, rows_at(s * G, G), :]
                else:
                    y1 = u1[key, l] + part[(b * NLONG + len(PAIRS) + l) * BUNDLE + i]
                y2 = z[key, l][M:] - LAM[l] * y1 if LAM[l] else z[key, l][M:]
                tmp[t, u * NB + l] = hold(qkv[t], u * NB + l, jnp.concatenate([z[key, l][:M], y1, y2], axis=0))

        def plain(t, h, k):
            lhs = jnp.concatenate([mem[k], hx[rows, tile(k)]], axis=0)
            _add(tmp, ("p", t, h), _dot(lhs, _unpack(wr[(t * H + h) * NB + k])))
            if k == NB - 1:
                tmp[t, h] = hold(qkv[t], h, tmp["p", t, h])

        def scores(h):
            sc = jnp.where(mask, _dot(tmp[0, h](), tmp[1, h](), NT) * scale, -1e9)
            e = jnp.exp(sc - jnp.max(sc, axis=-1, keepdims=True))
            eb[h] = e
            tmp["sum", h] = jnp.broadcast_to(jnp.sum(e, axis=-1, keepdims=True), (L, DH))

        def values(h):
            o = _dot(eb[h], tmp[2, h]()) * pltpu.reciprocal(tmp["sum", h], approx=True)
            tmp["o", h] = o
            u = h // NB
            if i is None:
                return
            if u == NU:
                tmp["o", h] = hold(ob, h, o)()
                return
            ob[i * H + h] = o
            if all(("o", u * NB + k) in tmp for k in range(NB)):
                o = [tmp["o", u * NB + k] for k in range(NB)]
                ev = {(k, l): jnp.concatenate([o[k][:M], _ev(o[k][M:], l)], axis=0) for k, l in ORDER}
                for k, l in ORDER:
                    tmp["o", u, k, l] = ev[k, l] - ev[l, l] if k != l else ev[l, l]

        def out(h, l):
            _add(tmp, ("y", l), _dot(tmp["o", h], _unpack(wo[l, h * 64:(h + 1) * 64, :])))

        run = dict(main=main, plain=plain, scores=scores, values=values, out=out, **extra)
        for op in ops:
            run[op[0]](*op[1:])

        cols = [tmp["y", l] for l in range(NB)]
        if i is not None:
            for l in range(NB):
                y2 = z["o", l][M:] - LAM[l] * u1["o", l] if LAM[l] else z["o", l][M:]
                cols[l] = jnp.concatenate([z["o", l][:M], u1["o", l], y2], axis=0) + cols[l]
        y = jnp.concatenate(cols, axis=1)
        memb[...] = y[:M]
        return xres[rows, :] + y[M:]

    def head_step(s, _):
        t = jnp.maximum(s // BUNDLE - 1, 0)
        for n in range(2):
            l = jnp.minimum(2 * (s % BUNDLE) + n, NB - 1)
            hb[t, rows_at(l * 128, 128), :] = xmid[rows_at(t * 128, 128), rows_at(l * 128, 128)].T
        share = pl.cdiv((NU - NG) * 8, HEAD * BUNDLE)
        for n in range(share):
            combine_out(jnp.minimum(NG * 8 + s * share + n, NU * 8 - 1))
        x = step(s, None, head_prog, {})
        ymid[rows_at((s % BUNDLE) * SEG, SEG), :] = x
        xmid[rows_at(s * SEG, SEG), :] = x
        prep_step(s + 1, 0)
        return 0

    def bundle(jb, _):
        extra = dict(long=lambda b, j: long_qkv(jb * BUNDLE, phase[b, j], BUNDLE, b, j),
                     long_out=functools.partial(long_out, jnp.maximum(jb - 1, 0), {}))
        for i in range(BUNDLE):
            s = jb * BUNDLE + i
            ymid[i * SEG:(i + 1) * SEG, :] = step(s, i, prog[i], extra)
            prep_step(s + 1, (i + 1) % BUNDLE)
        return 0

    def rounds(w1t, w2):
        w_loads = [pltpu.make_async_copy(src, dst, sems.at[3 + n]) for n, (src, dst) in enumerate(
            ((w1t_hbm, w1t.at[pl.ds(0, F)]), (w2_hbm, w2.at[pl.ds(0, F)]), (b1_hbm, b1_ref), (b2_hbm, b2_ref)))]
        for c in w_loads:
            c.start()
        for w in (w1t, w2):
            w[F:, :] = jnp.zeros((w.shape[0] - F, S), BF16)
        ST, FT = S // 128, w2.shape[0] // 128
        assert FT % MB in (0, 2)

        def mixer(it):
            def keep(n):
                return lambda i, v: hold(macc, n // MB % 3 * (2 * MB + 2) + i, v)

            b1 = b1_ref[...].astype(F32).reshape(1, F)
            b1 = jnp.concatenate([b1, jnp.zeros((1, FT * 128 - F), F32)], axis=1)
            b2 = b2_ref[...].astype(F32).reshape(1, S)
            up = [_mixer_lhs([_ln(hb[t + k], axis=0, twice=True) for k in range(MB)]) for t in range(0, ST, MB)]
            g = {}

            def hidden_tile(n, l, k):
                if n + MB <= FT:
                    return n + l
                return n + l % 2 if l // 2 == k // 2 else None

            def hidden(n):
                def activate(l, u):
                    t = hidden_tile(n, l, l)
                    if n + MB > FT and l < 2:
                        g[t] = u
                    else:
                        u = u + g[t] if t in g else u
                        g[t] = jax.nn.gelu(u + b1[:, tile(t)], approximate=True)

                def w(kt, k, l):
                    t = hidden_tile(n, l, k)
                    return None if t is None else w1t[tile(t), tile(kt * MB + k)]
                return _mixer_product(up, w, NT, keep(n), activate, first=n < 2 * MB)
            groups = [hidden(n) for n in range(0, FT, MB)]
            for _ in zip(*groups[:2]):
                pass
            for group in groups:
                for _ in group:
                    pass
            down = [_mixer_lhs([g[hidden_tile(n, k, k)] for k in range(MB)]) for n in range(0, FT, MB)]
            for n in range(0, ST, MB):
                def update(l, y):
                    t = n + l
                    x = xmid[tile(t), :] + (y + b2[:, tile(t)]).T
                    xres[tile(t), :] = x
                    xio[tile(t), :] = x.astype(BF16)
                    if t + 1 in STORES:
                        lo = STORES[STORES.index(t + 1) - 1]
                        rows = pl.ds(lo * 128, (t + 1 - lo) * 128)
                        copy = pltpu.make_async_copy(xio.at[rows], out_hbm.at[rows], sems.at[2])
                        if lo:
                            pl.when(it == 1)(copy.start)
                        else:
                            lax.fori_loop(0, it, lambda i, c: copy.start(), None)
                    if t < ST - LATE:
                        for i in range(BUNDLE):
                            prep_tokens(t * BUNDLE + i, x[i * SEG:(i + 1) * SEG])

                def w(kt, k, l):
                    t = hidden_tile(kt * MB, k, l)
                    return None if t is None else w2[tile(t), tile(n + l)]
                for _ in _mixer_product(down, w, NN, keep(n), update):
                    pass

        def restart():
            memb[...] = mem0_ref[...].astype(F32)
            prep_step(0, 0)

        def one_round(it, _):
            lax.fori_loop(jnp.where(it == 0, HEAD, 0), NBUN, bundle, 0)

            @pl.when(it == 0)
            def _():
                for c in w_loads:
                    c.wait()

            acc = {}
            for op in prog[0]:
                if op[0] == "long_out":
                    long_out(NBUN - 1, acc, *op[1:])
            mixer(it)

            @pl.when(it == 0)
            def _():
                for s in range((ST - LATE) * BUNDLE, NSEG):
                    prep_tokens(s, xres[rows_at(s * SEG, SEG), :])
                for (b, j), ph in phase.items():
                    if ph:
                        long_qkv(0, 0, ph, b, j)
                restart()
            return 0

        restart()
        lax.fori_loop(0, HEAD * BUNDLE, head_step, 0)
        lax.fori_loop(0, 2, one_round, 0)
        pltpu.make_async_copy(xio, out_hbm, sems.at[2]).wait()

    FP = pl.cdiv(F, 128) * 128
    pl.run_scoped(rounds, pltpu.VMEM((FP, S), BF16), pltpu.VMEM((FP, S), BF16))


@functools.partial(jax.jit, static_argnames=("A_seg_len",))
def pallas_interleave_layers__memory_aug_recurrent_mem_tr__mixer_token_mlp__prompt_kernel(
    A_x, A_mem0, A_Wq, A_Wk, A_Wv, A_Wo, A_seg_len, B_x, B_w1, B_b1, B_w2, B_b2,
):
    del B_x
    B, S, DM = A_x.shape
    H, DH = A_Wq.shape[1:]
    M = A_mem0.shape[1]
    SEG = int(A_seg_len)
    L = M + SEG
    G = SEG // 2
    NU = H // NB
    RB = BUNDLE * G
    assert (B, DM, H, DH, M, SEG) == (1, NB * 128, 32, 128, 8, 32) and S == STORES[-1] * 128
    hbm = pl.BlockSpec(memory_space=pl.ANY)
    V = pltpu.VMEM
    out = pl.pallas_call(
        _kernel,
        out_shape=jax.ShapeDtypeStruct((S, DM), A_x.dtype),
        grid=(1,),
        in_specs=[hbm] * 10,
        out_specs=hbm,
        scratch_shapes=[
            V((S, DM), BF16),
            V((S, DM), F32),
            V((S, DM), F32),
            V((S, DM), F32),
            V((NLONG, S // 4 + RB // 2, 128), U32),
            V((3 * H * NB, 64, 128), U32),
            V((NB, H * 64, 128), U32),
            V((4 * NU * NLONG, 64, 128), U32),
            V((3 * NU * NB, 64, 128), U32),
            V((NU * NB, 64, 128), U32),
            V((3 * NU * NB, HEAD * RB, 128), F32),
            V((3 * NU * NLONG * BUNDLE, G, 128), F32),
            V((NB, RB, 128), F32),
            V((M, DM), F32),
            V((NB * NB, M, 128), F32),
            V((BUNDLE * NB * NB, G, 128), F32),
            [V((H, L, DH), F32)] * 3,
            V((H, L, L), F32),
            V((BUNDLE * H, L, DH), F32),
            V((2 * NB, M + G, 128), F32),
            V((BUNDLE * SEG, DM), F32),
            V((S // 128, DM, 128), F32),
            V((6 * MB + 6, DM // 2, 128), F32),
            V((M, DM), A_mem0.dtype),
            V(B_b1.shape, B_b1.dtype),
            V(B_b2.shape, B_b2.dtype),
            pltpu.SemaphoreType.DMA((14 + 2 * NB,)),
        ],
        compiler_params=pltpu.CompilerParams(vmem_limit_bytes=126 * 2**20),
        name="rmt_mixer",
    )(
        A_x.reshape(S, DM), A_mem0.reshape(M, DM), A_Wq, A_Wk, A_Wv, A_Wo.reshape(H * DH, DM),
        B_w1.T, B_b1, B_w2, B_b2,
    )
    return out.reshape(B, S, DM)
```
